```python
import jax
import jax.numpy as jnp

def _softmax(x, axis=-1):
    return jax.nn.softmax(x, axis=axis)

def _gelu(x):
    return jax.nn.gelu(x, approximate=True)

def _silu(x):
    return jax.nn.silu(x)

def _sigmoid(x):
    return jax.nn.sigmoid(x)

def _layernorm(x, axis=-1, eps=1e-05):
    m = jnp.mean(x, axis=axis, keepdims=True)
    v = jnp.var(x, axis=axis, keepdims=True)
    return (x - m) / jnp.sqrt(v + eps)

def _scatter_add(tgt, idx, src, axis=0):
    return tgt.at[idx].add(src)

def _segment_sum(src, seg, n):
    return jax.ops.segment_sum(src, seg, n)

class _Rng:

    def __init__(self, key):
        self._k = key

    def _next(self):
        self._k, sub = jax.random.split(self._k)
        return sub

    def normal(self, shape):
        return jax.random.normal(self._next(), shape, dtype=jnp.bfloat16)

    def randint(self, lo, hi, shape):
        return jax.random.randint(self._next(), shape, lo, hi, dtype=jnp.int32)

    def uniform(self, shape, lo=0.0, hi=1.0):
        return jax.random.uniform(self._next(), shape, jnp.bfloat16, lo, hi)

    def permutation(self, n):
        return jax.random.permutation(self._next(), n)
kernel_name = 'interleave_layers__sliding_local_dilated__mixer_gmlp__prompt'

def setup_inputs():
    _rng = _Rng(jax.random.key(int.from_bytes(__import__("os").urandom(4), "little")))
    _w = lambda a: (lambda t: t.astype(jnp.bfloat16) if jnp.issubdtype(t.dtype, jnp.floating) else t)(jnp.asarray(a))

    def _A_setup():
        B, S, D = (1, 2048, 576)
        return {'x': _w((lambda *s: _rng.normal(s) * 0.05)(B, S, D)), 'wqkv': _w((lambda *s: _rng.normal(s) * 0.05)(D, 3 * D)), 'wo': _w((lambda *s: _rng.normal(s) * 0.05)(D, D))}
    _A_in = _A_setup()

    def _B_setup():
        B, S, D, F = (1, 2048, 576, 4608)
        Fh = F // 2
        return {'x': _w((lambda *s: _rng.normal(s) * 0.05)(B, S, D)), 'w_in': _w((lambda *s: _rng.normal(s) * 0.05)(D, 2 * Fh)), 'w_sp': _w(0.01 * (lambda *s: _rng.normal(s) * 0.05)(S, S)), 'b_sp': _w(1.0 + 0.01 * (lambda *s: _rng.normal(s) * 0.05)(S)), 'w_out': _w((lambda *s: _rng.normal(s) * 0.05)(Fh, D))}
    _B_in = _B_setup()
    return {'A_x': _A_in['x'], 'A_wqkv': _A_in['wqkv'], 'A_wo': _A_in['wo'], 'B_x': _B_in['x'], 'B_w_in': _B_in['w_in'], 'B_w_sp': _B_in['w_sp'], 'B_b_sp': _B_in['b_sp'], 'B_w_out': _B_in['w_out']}

def reference(A_x, A_wqkv, A_wo, B_x, B_w_in, B_w_sp, B_b_sp, B_w_out):

    def _A_ref(x, wqkv, wo):
        B, S, D = x.shape
        H = 32
        Dh = D // H
        W, dil = (8, 2)
        qkv = (lambda x, *d: x.transpose(*d))((x @ wqkv).reshape(B, S, 3, H, Dh), 2, 0, 3, 1, 4)
        q, k, v = (qkv[0], qkv[1], qkv[2])
        scale = Dh ** (-0.5)
        pos = jnp.arange(S)
        off = jnp.arange(W) * dil
        idx = pos[:, None] - off[None, :]
        mask = idx >= 0
        idx_c = jnp.where(mask, idx, 0).reshape(-1)
        kg = k[:, :, idx_c, :].reshape(B, H, S, W, Dh)
        vg = v[:, :, idx_c, :].reshape(B, H, S, W, Dh)
        logits = jnp.einsum('bhsd,bhswd->bhsw', q, kg) * scale
        logits = jnp.where(mask[None, None, :, :], logits, -1000000000.0)
        attn = _softmax(logits, axis=-1)
        o = jnp.einsum('bhsw,bhswd->bhsd', attn, vg)
        return (lambda x, *d: x.transpose(*d))(o, 0, 2, 1, 3).reshape(B, S, D) @ wo

    def _B_ref(x, w_in, w_sp, b_sp, w_out):
        B, S, D = x.shape
        F = w_in.shape[-1]
        Fh = F // 2
        z = _gelu(jnp.einsum('bsd,df->bsf', x, w_in))
        z1 = z[..., :Fh].copy()
        z2 = _layernorm(z[..., Fh:], axis=-1)
        g = jnp.einsum('ts,bsf->btf', w_sp, z2) + b_sp[None, :, None]
        return jnp.einsum('bsf,fd->bsd', z1 * g, w_out)
    x = A_x
    x = x + _A_ref(_layernorm(x, axis=-1), A_wqkv, A_wo)
    x = x + _B_ref(_layernorm(x, axis=-1), B_w_in, B_w_sp, B_b_sp, B_w_out)
    x = x + _A_ref(_layernorm(x, axis=-1), A_wqkv, A_wo)
    x = x + _B_ref(_layernorm(x, axis=-1), B_w_in, B_w_sp, B_b_sp, B_w_out)
    return x
```

```python
import jax
import jax.numpy as jnp
import jax.experimental.pallas as pl
import jax.experimental.pallas.tpu as pltpu

S, D, DP, H, DH, FH = 2048, 576, 640, 32, 18, 2304
T1, T2, C, HALO = 256, 512, 64, 16
F32, BF = jnp.float32, jnp.bfloat16


def _ln(x):
    m = jnp.mean(x, axis=-1, keepdims=True)
    c = x - m
    v = jnp.mean(c * c, axis=-1, keepdims=True)
    return c * jax.lax.rsqrt(v + 1e-5)


def _dot(a, b):
    return jnp.dot(a, b, preferred_element_type=F32)


def _kernel(x_ref, wqkv_ref, wo_ref, b_ref, win_h, wsp_h, wout_h, o_ref,
            win, wsp, wout, wq, wo, xs, z1, z2, qs, ks, vs, os_, sem):
    cps = [pltpu.make_async_copy(a, b, sem.at[i])
           for i, (a, b) in enumerate(((win_h, win), (wsp_h, wsp), (wout_h, wout)))]
    for c in cps:
        c.start()
    r = jax.lax.broadcasted_iota(jnp.int32, (D, DP), 0)
    c = jax.lax.broadcasted_iota(jnp.int32, (D, DP), 1)
    P = jnp.where((r == (c & 31) * DH + (c >> 5)) & (c < D), 1.0, 0.0).astype(BF)
    for i in range(3):
        wq[:, i * DP:(i + 1) * DP] = _dot(wqkv_ref[:, i * D:(i + 1) * D], P).astype(BF)
    r = jax.lax.broadcasted_iota(jnp.int32, (DP, D), 0)
    c = jax.lax.broadcasted_iota(jnp.int32, (DP, D), 1)
    PT = jnp.where((c == (r & 31) * DH + (r >> 5)) & (r < D), 1.0, 0.0).astype(BF)
    wo[...] = _dot(PT, wo_ref[...]).astype(BF)
    xs[...] = x_ref[...].astype(F32)
    cps[0].wait()

    def part1(i, _):
        rows = pl.ds(pl.multiple_of(i * T1, T1), T1)
        x = xs[rows, :]
        qkv = _dot(_ln(x).astype(BF), wq[...])
        qs[...] = qkv[:, :DP] * (DH ** -0.5)
        ks[HALO:, :] = qkv[:, DP:2 * DP]
        vs[HALO:, :] = qkv[:, 2 * DP:]
        for j in range(T1 // C):
            pos = i * T1 + j * C + jax.lax.broadcasted_iota(jnp.int32, (C, 128), 0)
            ls = []
            for w in range(8):
                o = HALO + j * C - 2 * w
                a = None
                for t in range(5):
                    ln = slice(t * 128, t * 128 + 128)
                    p = qs[j * C:(j + 1) * C, ln] * ks[o:o + C, ln]
                    a = p if a is None else a + p
                a = a + pltpu.roll(a, 64, 1)
                a = a + pltpu.roll(a, 32, 1)
                ls.append(jnp.where(pos >= 2 * w, a, -1e9) if w else a)
            m = ls[0]
            for l in ls[1:]:
                m = jnp.maximum(m, l)
            es = [jnp.exp(l - m) for l in ls]
            inv = 1.0 / sum(es[1:], es[0])
            es = [e * inv for e in es]
            for t in range(5):
                ln = slice(t * 128, t * 128 + 128)
                a = None
                for w in range(8):
                    o = HALO + j * C - 2 * w
                    p = es[w] * vs[o:o + C, ln]
                    a = p if a is None else a + p
                os_[j * C:(j + 1) * C, ln] = a.astype(BF)
        ks[:HALO, :] = ks[T1:, :]
        vs[:HALO, :] = vs[T1:, :]
        x = x + _dot(os_[...], wo[...])
        xs[rows, :] = x
        h = _ln(x).astype(BF)
        z2[rows, :] = _ln(jax.nn.gelu(_dot(h, win[:, FH:]), approximate=True)).astype(BF)
        z1[rows, :] = jax.nn.gelu(_dot(h, win[:, :FH]), approximate=True).astype(BF)
        return 0

    def part2(i, _):
        rows = pl.ds(pl.multiple_of(i * T2, T2), T2)
        g = _dot(wsp[rows, :], z2[...]) + b_ref[rows, :].astype(F32)
        u = (z1[rows, :].astype(F32) * g).astype(BF)
        xs[rows, :] = xs[rows, :] + _dot(u, wout[...])
        return 0

    def layer(l, _):
        ks[:HALO, :] = jnp.zeros((HALO, DP), F32)
        vs[:HALO, :] = jnp.zeros((HALO, DP), F32)
        jax.lax.fori_loop(0, S // T1, part1, 0)

        @pl.when(l == 0)
        def _():
            cps[1].wait()
            cps[2].wait()
        jax.lax.fori_loop(0, S // T2, part2, 0)
        return 0

    jax.lax.fori_loop(0, 2, layer, 0)
    o_ref[...] = xs[...].astype(o_ref.dtype)


@jax.jit
def pallas_interleave_layers__sliding_local_dilated__mixer_gmlp__prompt_kernel(
        A_x, A_wqkv, A_wo, B_x, B_w_in, B_w_sp, B_b_sp, B_w_out):
    V = pltpu.VMEM
    vm = pl.BlockSpec(memory_space=V)
    hb = pl.BlockSpec(memory_space=pl.ANY)
    out = pl.pallas_call(
        _kernel,
        in_specs=[vm] * 4 + [hb] * 3,
        out_specs=vm,
        out_shape=jax.ShapeDtypeStruct((S, D), A_x.dtype),
        scratch_shapes=[
            V((D, 2 * FH), BF), V((S, S), BF), V((FH, D), BF),
            V((D, 3 * DP), BF), V((DP, D), BF), V((S, D), F32),
            V((S, FH), BF), V((S, FH), BF),
            V((T1, DP), F32), V((T1 + HALO, DP), F32), V((T1 + HALO, DP), F32),
            V((T1, DP), BF), pltpu.SemaphoreType.DMA((3,))],
        compiler_params=pltpu.CompilerParams(vmem_limit_bytes=110 * 2**20),
    )(A_x.reshape(S, D), A_wqkv, A_wo, B_b_sp.reshape(S, 1), B_w_in, B_w_sp, B_w_out)
    return out.reshape(1, S, D)
```

```python
import jax
import jax.numpy as jnp
import jax.experimental.pallas as pl
import jax.experimental.pallas.tpu as pltpu

S, D, DP, H, DH, FH = 2048, 576, 640, 32, 18, 2304
T1, T2, C, HALO = 256, 512, 64, 16
F32, BF = jnp.float32, jnp.bfloat16


def _ln(x):
    m = jnp.mean(x, axis=-1, keepdims=True)
    c = x - m
    v = jnp.mean(c * c, axis=-1, keepdims=True)
    return c * jax.lax.rsqrt(v + 1e-5)


def _dot(a, b):
    return jnp.dot(a, b, preferred_element_type=F32)


def _kernel(x_ref, wqkv_ref, wo_ref, b_ref, win_h, wsp_h, wout_h, o_ref,
            win, wsp, wout, wq, wo, xs, z1, z2, qs, ks, vs, os_, hs, bs, woT, sem):
    cps = [pltpu.make_async_copy(a, b, sem.at[i])
           for i, (a, b) in enumerate(((win_h, win), (wsp_h, wsp), (wout_h, woT)))]
    for c in cps:
        c.start()
    r = jax.lax.broadcasted_iota(jnp.int32, (D, DP), 0)
    c = jax.lax.broadcasted_iota(jnp.int32, (D, DP), 1)
    P = jnp.where((r == (c & 31) * DH + (c >> 5)) & (c < D), 1.0, 0.0).astype(BF)
    for i in range(3):
        wq[:, i * DP:(i + 1) * DP] = _dot(wqkv_ref[:, i * D:(i + 1) * D], P).astype(BF)
    r = jax.lax.broadcasted_iota(jnp.int32, (DP, D), 0)
    c = jax.lax.broadcasted_iota(jnp.int32, (DP, D), 1)
    PT = jnp.where((c == (r & 31) * DH + (r >> 5)) & (r < D), 1.0, 0.0).astype(BF)
    wo[...] = _dot(PT, wo_ref[...]).astype(BF)
    xs[...] = x_ref[...].astype(F32).T
    bs[...] = jnp.broadcast_to(b_ref[...].astype(F32), (128, S)).T

    def attn(i):
        rows = pl.ds(pl.multiple_of(i * T1, T1), T1)
        x = xs[rows, :]
        qkv = _dot(_ln(x).astype(BF), wq[...])
        qs[...] = qkv[:, :DP] * (DH ** -0.5)
        ks[HALO:, :] = qkv[:, DP:2 * DP]
        vs[HALO:, :] = qkv[:, 2 * DP:]
        for j in range(T1 // C):
            pos = i * T1 + j * C + jax.lax.broadcasted_iota(jnp.int32, (C, 128), 0)
            ls = []
            for w in range(8):
                o = HALO + j * C - 2 * w
                a = None
                for t in range(5):
                    ln = slice(t * 128, t * 128 + 128)
                    p = qs[j * C:(j + 1) * C, ln] * ks[o:o + C, ln]
                    a = p if a is None else a + p
                a = a + pltpu.roll(a, 64, 1)
                a = a + pltpu.roll(a, 32, 1)
                ls.append(jnp.where(pos >= 2 * w, a, -1e9) if w else a)
            m = ls[0]
            for l in ls[1:]:
                m = jnp.maximum(m, l)
            es = [jnp.exp(l - m) for l in ls]
            inv = 1.0 / sum(es[1:], es[0])
            es = [e * inv for e in es]
            for t in range(5):
                ln = slice(t * 128, t * 128 + 128)
                a = None
                for w in range(8):
                    o = HALO + j * C - 2 * w
                    p = es[w] * vs[o:o + C, ln]
                    a = p if a is None else a + p
                os_[j * C:(j + 1) * C, ln] = a.astype(BF)
        ks[:HALO, :] = ks[T1:, :]
        vs[:HALO, :] = vs[T1:, :]
        x = x + _dot(os_[...], wo[...])
        xs[rows, :] = x
        return _ln(x).astype(BF)

    def ffn(i, h):
        rows = pl.ds(pl.multiple_of(i * T1, T1), T1)
        z2[rows, :] = _ln(jax.nn.gelu(_dot(h, win[:, FH:]), approximate=True)).astype(BF)
        z1[rows, :] = jax.nn.gelu(_dot(h, win[:, :FH]), approximate=True).astype(BF)

    def part1(i, _):
        h = hs[...]
        hn = attn(i + 1)
        ffn(i, h)
        hs[...] = hn
        return 0

    def part2(i, _):
        rows = pl.ds(pl.multiple_of(i * T2, T2), T2)
        g = _dot(wsp[rows, :], z2[...]) + bs[rows, :1]
        u = (z1[rows, :].astype(F32) * g).astype(BF)
        xs[rows, :] = xs[rows, :] + _dot(u, wout[...])
        return 0

    def layer(l, _):
        ks[:HALO, :] = jnp.zeros((HALO, DP), F32)
        vs[:HALO, :] = jnp.zeros((HALO, DP), F32)
        hs[...] = attn(0)

        @pl.when(l == 0)
        def _():
            cps[0].wait()
        jax.lax.fori_loop(0, S // T1 - 1, part1, 0)
        ffn(S // T1 - 1, hs[...])

        @pl.when(l == 0)
        def _():
            cps[1].wait()
            cps[2].wait()
            wout[...] = woT[...].T
        jax.lax.fori_loop(0, S // T2, part2, 0)
        return 0

    jax.lax.fori_loop(0, 2, layer, 0)
    o_ref[...] = xs[...].T.astype(o_ref.dtype)


@jax.jit
def pallas_interleave_layers__sliding_local_dilated__mixer_gmlp__prompt_kernel(
        A_x, A_wqkv, A_wo, B_x, B_w_in, B_w_sp, B_b_sp, B_w_out):
    V = pltpu.VMEM
    vm = pl.BlockSpec(memory_space=V)
    hb = pl.BlockSpec(memory_space=pltpu.HBM)
    out = pl.pallas_call(
        _kernel,
        in_specs=[vm] * 4 + [hb] * 3,
        out_specs=vm,
        out_shape=jax.ShapeDtypeStruct((D, S), A_x.dtype),
        scratch_shapes=[
            V((D, 2 * FH), BF), V((S, S), BF), V((FH, D), BF),
            V((D, 3 * DP), BF), V((DP, D), BF), V((S, D), F32),
            V((S, FH), BF), V((S, FH), BF),
            V((T1, DP), F32), V((T1 + HALO, DP), F32), V((T1 + HALO, DP), F32),
            V((T1, DP), BF), V((T1, D), BF), V((S, 128), F32), V((D, FH), BF), pltpu.SemaphoreType.DMA((3,))],
        compiler_params=pltpu.CompilerParams(vmem_limit_bytes=110 * 2**20),
    )(A_x.reshape(S, D).T, A_wqkv, A_wo, B_b_sp.reshape(1, S), B_w_in, B_w_sp, B_w_out.T)
    return out.T.reshape(1, S, D)
```

```python
import jax
import jax.numpy as jnp
import jax.experimental.pallas as pl
import jax.experimental.pallas.tpu as pltpu

S, D, DP, H, DH, FH = 2048, 576, 640, 32, 18, 2304
T1, T2, C, HALO = 256, 512, 128, 16
F32, BF = jnp.float32, jnp.bfloat16


def _ln(x):
    m = jnp.mean(x, axis=-1, keepdims=True)
    c = x - m
    v = jnp.mean(c * c, axis=-1, keepdims=True)
    return c * jax.lax.rsqrt(v + 1e-5)


def _dot(a, b):
    return jnp.dot(a, b, preferred_element_type=F32)


def _kernel(x_ref, wqkv_ref, wo_ref, b_ref, win_h, wsp_h, wout_h, o_ref,
            win, wsp, wq, wo, xs, z1, z2, qs, ks, vs, os_, hs, bs, woT, sem):
    cps = [pltpu.make_async_copy(a, b, sem.at[i])
           for i, (a, b) in enumerate(((win_h, win), (wsp_h, wsp), (wout_h, woT)))]
    for c in cps:
        c.start()
    r = jax.lax.broadcasted_iota(jnp.int32, (D, DP), 0)
    c = jax.lax.broadcasted_iota(jnp.int32, (D, DP), 1)
    P = jnp.where((r == (c & 31) * DH + (c >> 5)) & (c < D), 1.0, 0.0).astype(BF)
    for i in range(3):
        wq[:, i * DP:(i + 1) * DP] = _dot(wqkv_ref[:, i * D:(i + 1) * D], P).astype(BF)
    r = jax.lax.broadcasted_iota(jnp.int32, (DP, D), 0)
    c = jax.lax.broadcasted_iota(jnp.int32, (DP, D), 1)
    PT = jnp.where((c == (r & 31) * DH + (r >> 5)) & (r < D), 1.0, 0.0).astype(BF)
    wo[...] = _dot(PT, wo_ref[...]).astype(BF)
    xs[...] = x_ref[...].astype(F32).T
    bs[...] = jnp.broadcast_to(b_ref[...].astype(F32), (128, S)).T

    def attn(i):
        rows = pl.ds(pl.multiple_of(i * T1, T1), T1)
        x = xs[rows, :]
        qkv = _dot(_ln(x).astype(BF), wq[...])
        qs[...] = qkv[:, :DP] * (DH ** -0.5)
        ks[HALO:, :] = qkv[:, DP:2 * DP]
        vs[HALO:, :] = qkv[:, 2 * DP:]
        for j in range(T1 // C):
            pos = i * T1 + j * C + jax.lax.broadcasted_iota(jnp.int32, (C, 128), 0)
            ls = []
            for w in range(8):
                o = HALO + j * C - 2 * w
                a = None
                for t in range(5):
                    ln = slice(t * 128, t * 128 + 128)
                    p = qs[j * C:(j + 1) * C, ln] * ks[o:o + C, ln]
                    a = p if a is None else a + p
                a = a + pltpu.roll(a, 64, 1)
                a = a + pltpu.roll(a, 32, 1)
                ls.append(jnp.where(pos >= 2 * w, a, -1e9) if w else a)
            m = ls[0]
            for l in ls[1:]:
                m = jnp.maximum(m, l)
            es = [jnp.exp(l - m) for l in ls]
            inv = 1.0 / sum(es[1:], es[0])
            es = [e * inv for e in es]
            for t in range(5):
                ln = slice(t * 128, t * 128 + 128)
                a = None
                for w in range(8):
                    o = HALO + j * C - 2 * w
                    p = es[w] * vs[o:o + C, ln]
                    a = p if a is None else a + p
                os_[j * C:(j + 1) * C, ln] = a.astype(BF)
        ks[:HALO, :] = ks[T1:, :]
        vs[:HALO, :] = vs[T1:, :]
        x = x + _dot(os_[...], wo[...])
        xs[rows, :] = x
        return _ln(x).astype(BF)

    def ffn(i, h):
        rows = pl.ds(pl.multiple_of(i * T1, T1), T1)
        z2[rows, :] = _ln(jax.nn.gelu(_dot(h, win[:, FH:]), approximate=True)).astype(BF)
        z1[rows, :] = jax.nn.gelu(_dot(h, win[:, :FH]), approximate=True).astype(BF)

    def part1(i, _):
        h = hs[...]
        hn = attn(i + 1)
        ffn(i, h)
        hs[...] = hn
        return 0

    def part2(i, _):
        rows = pl.ds(pl.multiple_of(i * T2, T2), T2)
        g = _dot(wsp[rows, :], z2[...]) + bs[rows, :1]
        u = (z1[rows, :].astype(F32) * g).astype(BF)
        xs[rows, :] = xs[rows, :] + jax.lax.dot_general(woT[...], u, (((1,), (1,)), ((), ())), preferred_element_type=F32).T
        return 0

    def layer(l, _):
        ks[:HALO, :] = jnp.zeros((HALO, DP), F32)
        vs[:HALO, :] = jnp.zeros((HALO, DP), F32)
        hs[...] = attn(0)

        @pl.when(l == 0)
        def _():
            cps[0].wait()
        jax.lax.fori_loop(0, S // T1 - 1, part1, 0)
        ffn(S // T1 - 1, hs[...])

        @pl.when(l == 0)
        def _():
            cps[1].wait()
            cps[2].wait()
        jax.lax.fori_loop(0, S // T2, part2, 0)
        return 0

    jax.lax.fori_loop(0, 2, layer, 0)
    o_ref[...] = xs[...].T.astype(o_ref.dtype)


@jax.jit
def pallas_interleave_layers__sliding_local_dilated__mixer_gmlp__prompt_kernel(
        A_x, A_wqkv, A_wo, B_x, B_w_in, B_w_sp, B_b_sp, B_w_out):
    V = pltpu.VMEM
    vm = pl.BlockSpec(memory_space=V)
    hb = pl.BlockSpec(memory_space=pltpu.HBM)
    out = pl.pallas_call(
        _kernel,
        in_specs=[vm] * 4 + [hb] * 3,
        out_specs=vm,
        out_shape=jax.ShapeDtypeStruct((D, S), A_x.dtype),
        scratch_shapes=[
            V((D, 2 * FH), BF), V((S, S), BF),
            V((D, 3 * DP), BF), V((DP, D), BF), V((S, D), F32),
            V((S, FH), BF), V((S, FH), BF),
            V((T1, DP), F32), V((T1 + HALO, DP), F32), V((T1 + HALO, DP), F32),
            V((T1, DP), BF), V((T1, D), BF), V((S, 128), F32), V((D, FH), BF), pltpu.SemaphoreType.DMA((3,))],
        compiler_params=pltpu.CompilerParams(vmem_limit_bytes=110 * 2**20),
    )(A_x.reshape(S, D).T, A_wqkv, A_wo, B_b_sp.reshape(1, S), B_w_in, B_w_sp, B_w_out.T)
    return out.T.reshape(1, S, D)
```
